```python
import os as _os
_os.environ.setdefault("JAX_PLATFORMS", "cpu")
import jax
import jax.numpy as jnp

def _softmax(x, axis=-1):
    return jax.nn.softmax(x, axis=axis)
def _gelu(x):
    return jax.nn.gelu(x, approximate=True)
def _silu(x):
    return jax.nn.silu(x)
def _sigmoid(x):
    return jax.nn.sigmoid(x)
def _layernorm(x, axis=-1, eps=1e-5):
    m = jnp.mean(x, axis=axis, keepdims=True)
    v = jnp.var(x, axis=axis, keepdims=True)
    return (x - m) / jnp.sqrt(v + eps)
def _scatter_add(tgt, idx, src, axis=0):
    return tgt.at[idx].add(src)
def _segment_sum(src, seg, n):
    return jax.ops.segment_sum(src, seg, n)
class _Rng:
    def __init__(self, key):
        self._k = key
    def _next(self):
        self._k, sub = jax.random.split(self._k)
        return sub
    def normal(self, shape):
        return jax.random.normal(self._next(), shape, dtype=jnp.bfloat16)
    def randint(self, lo, hi, shape):
        return jax.random.randint(self._next(), shape, lo, hi, dtype=jnp.int32)
    def uniform(self, shape, lo=0.0, hi=1.0):
        return jax.random.uniform(self._next(), shape, jnp.bfloat16, lo, hi)
    def permutation(self, n):
        return jax.random.permutation(self._next(), n)


kernel_name = 'concat_heads__mha_block__linear_attn_block__prompt'

def setup_inputs():
    _rng = _Rng(jax.random.key(int.from_bytes(__import__("os").urandom(4), "little")))
    _w = (lambda a: (lambda t: t.astype(jnp.bfloat16) if jnp.issubdtype(t.dtype, jnp.floating) else t)(jnp.asarray(a)))
    def _A_setup():
        B, S, D, H = 1, 2048, 1024, 32
        return {
            "x": _w((lambda *s: _rng.normal(s) * 0.2)(B, S, D)),
            "wqkv": _w((lambda *s: _rng.normal(s) * 0.2)(D, 3 * D)),
            "wo": _w((lambda *s: _rng.normal(s) * 0.05)(D, D)),
        }
    _A_in = _A_setup()

    def _B_setup():
        B, S, D = 1, 2048, 1024
        return {
            "x": _w((lambda *s: _rng.normal(s) * 0.05)(B, S, D)),
            "wqkv": _w((lambda *s: _rng.normal(s) * 1.6)(D, 3 * D)),
            "wo": _w((lambda *s: _rng.normal(s) * 0.1)(D, D)),
        }
    _B_in = _B_setup()

    return {
        "A_x": _A_in["x"],
        "A_wqkv": _A_in["wqkv"],
        "A_wo": _A_in["wo"],
        "B_x": _B_in["x"],
        "B_wqkv": _B_in["wqkv"],
        "B_wo": _B_in["wo"],
    }

def reference(A_x, A_wqkv, A_wo, B_x, B_wqkv, B_wo):
    def _A_ref(x, wqkv, wo):
        B, S, D = x.shape
        H = 32
        Dh = D // H
        qkv = (lambda x, *d: x.transpose(*d))((x @ wqkv).reshape(B, S, 3, H, Dh), 2, 0, 3, 1, 4)
        q, k, v = qkv[0], qkv[1], qkv[2]
        scores = jnp.einsum("bhqd,bhkd->bhqk", q, k) * (Dh ** -0.5)
        p = _softmax(scores, axis=-1)
        o = jnp.einsum("bhqk,bhkd->bhqd", p, v)
        return (lambda x, *d: x.transpose(*d))(o, 0, 2, 1, 3).reshape(B, S, D) @ wo

    def _B_ref(x, wqkv, wo):
        B, S, D = x.shape
        H = 32; Dh = D // H
        qkv = (lambda x, *d: x.transpose(*d))((x @ wqkv).reshape(B, S, 3, H, Dh), 2, 0, 3, 1, 4)
        q, k, v = qkv[0], qkv[1], qkv[2]
        phi = lambda t: jnp.where(t > 0, t + 1, jnp.exp(t)) + 1e-6
        pq, pk = phi(q), phi(k)
        kv = jnp.einsum("bhsd,bhse->bhde", pk, v)
        z = jnp.einsum("bhsd->bhd", pk)
        num = jnp.einsum("bhqd,bhde->bhqe", pq, kv)
        den = jnp.einsum("bhqd,bhd->bhq", pq, z)[..., None] + 1e-6
        o = num / den
        return (lambda x, *d: x.transpose(*d))(o, 0, 2, 1, 3).reshape(B, S, D) @ wo

    a = _A_ref(A_x, A_wqkv, A_wo)
    b = _B_ref(B_x, B_wqkv, B_wo)
    return jnp.concatenate([a, b], axis=-1)
```

```python
import math

import jax
import jax.numpy as jnp
from jax import lax
import jax.experimental.pallas as pl
import jax.experimental.pallas.tpu as pltpu

_H = 32
_LANES = 128
_BQ = 512
_CK = 128
_RB = 512
_CB = 512

_NT = (((1,), (1,)), ((), ()))
_TN = (((0,), (0,)), ((), ()))
_TT = (((0,), (1,)), ((), ()))


def _dot(a, b, dims=None):
    if dims is None:
        return jnp.dot(a, b, preferred_element_type=jnp.float32)
    return lax.dot_general(a, b, dims, preferred_element_type=jnp.float32)


def _phi(t):
    return jnp.where(t > 0, t + 1.0, jnp.exp(t)) + 1e-6


def _kernel(xa_hbm, wa_hbm, woa_hbm, xb_hbm, wb_hbm, wob_hbm, out_hbm,
            xa, wa, woa, xb, wb, wob,
            q_s, k_s, vt_s, ot_s, sa_s, sb_s, vb_s, out_s,
            in_sems, out_sems):
    S, D = xa.shape
    dh = D // _H
    hpg = _LANES // dh
    ngrp = D // _LANES
    nr = S // _RB
    ncb = D // _CB
    gpb = _CB // _LANES
    nq = S // _BQ
    bf16, f32 = jnp.bfloat16, jnp.float32

    def x_copy(r):
        rows = pl.ds(r * _RB, _RB)
        return pltpu.make_async_copy(xa_hbm.at[rows, :], xa.at[rows, :], in_sems.at[r])

    def w_copy(c):
        cols = pl.ds(c * _CB, _CB)
        return pltpu.make_async_copy(wa_hbm.at[:, cols], wa.at[:, cols], in_sems.at[nr + c])

    rest = [
        pltpu.make_async_copy(src, dst, in_sems.at[nr + 3 * ncb + i])
        for i, (src, dst) in enumerate(
            [(woa_hbm, woa), (xb_hbm, xb), (wb_hbm, wb), (wob_hbm, wob)])
    ]
    x_copy(0).start()
    w_copy(0).start()
    for r in range(1, nr):
        x_copy(r).start()
    for c in range(1, 3 * ncb):
        w_copy(c).start()
    for cp in rest:
        cp.start()

    qscale = (dh ** -0.5) * math.log2(math.e)

    def store_groups(dst, c, rows, val):
        for g in range(gpb):
            dst[c * gpb + g, rows, :] = val[:, g * _LANES:(g + 1) * _LANES]

    for c in range(3 * ncb):
        w_copy(c).wait()
        part, cc = divmod(c, ncb)
        cols = slice(c * _CB, (c + 1) * _CB)

        def proj_a(r, carry, part=part, cc=cc, cols=cols):
            rows = pl.ds(pl.multiple_of(r * _RB, _RB), _RB)
            if part == 0:
                store_groups(q_s, cc, rows, (_dot(xa[rows, :], wa[:, cols]) * qscale).astype(bf16))
            elif part == 1:
                store_groups(k_s, cc, rows, _dot(xa[rows, :], wa[:, cols]).astype(bf16))
            else:
                vt = _dot(wa[:, cols], xa[rows, :], _TT)
                vt_s[cc * _CB:(cc + 1) * _CB, rows] = vt.astype(bf16)
            return carry

        if c == 0:
            for r in range(nr):
                x_copy(r).wait()
                proj_a(r, 0)
        else:
            lax.fori_loop(0, nr, proj_a, 0)

    lane = lax.broadcasted_iota(jnp.int32, (_BQ, _LANES), 1)
    n_it = _H * nq

    def masked_q(it):
        h = it // nq
        qi = it % nq
        q = q_s[h // hpg, pl.ds(pl.multiple_of(qi * _BQ, _BQ), _BQ), :]
        return jnp.where(lane // dh == h % hpg, q, jnp.zeros_like(q))

    def attn_step(it, m_cur, s_cur, s_nxt):
        h = it // nq
        qi = it % nq
        nxt = jnp.minimum(it + 1, n_it - 1)
        qm = masked_q(nxt)
        gn = nxt // nq // hpg
        hs = pl.ds(pl.multiple_of(h * dh, dh), dh)
        m8 = l8 = acc = None
        for c in range(S // _CK):
            ks = slice(c * _CK, (c + 1) * _CK)
            st = _dot(k_s[gn, ks, :], qm, _NT)
            s_nxt[ks, :] = st
            mm = jnp.max(st.reshape(_CK // 8, 8, _BQ), axis=0)
            m8 = mm if m8 is None else jnp.maximum(m8, mm)
            p = jnp.exp2(s_cur[ks, :] - m_cur)
            ll = jnp.sum(p.reshape(_CK // 8, 8, _BQ), axis=0)
            l8 = ll if l8 is None else l8 + ll
            a = _dot(vt_s[hs, ks], p.astype(bf16))
            acc = a if acc is None else acc + a
        l = jnp.sum(l8, axis=0, keepdims=True)
        ot_s[hs, pl.ds(pl.multiple_of(qi * _BQ, _BQ), _BQ)] = (acc / l).astype(bf16)
        return jnp.max(m8, axis=0, keepdims=True)

    st0 = _dot(k_s[0], masked_q(0), _NT)
    sa_s[...] = st0
    m0 = jnp.max(st0, axis=0, keepdims=True)

    def attn_pair(j, m):
        m = attn_step(2 * j, m, sa_s, sb_s)
        return attn_step(2 * j + 1, m, sb_s, sa_s)

    lax.fori_loop(0, n_it // 2, attn_pair, m0)

    def out_copy(half, r):
        rows = pl.ds(r * _RB, _RB)
        cols = pl.ds(half * D, D)
        return pltpu.make_async_copy(out_s.at[rows, cols], out_hbm.at[rows, cols],
                                     out_sems.at[half * nr + r])

    rest[0].wait()
    for r in range(nr):
        rows = slice(r * _RB, (r + 1) * _RB)
        out_s[rows, 0:D] = _dot(ot_s[:, rows], woa[...], _TN).astype(bf16)
        out_copy(0, r).start()

    rest[1].wait()
    rest[2].wait()
    for c in range(3 * ncb):
        part, cc = divmod(c, ncb)
        cols = slice(c * _CB, (c + 1) * _CB)

        def proj_b(r, carry, part=part, cc=cc, cols=cols):
            rows = pl.ds(pl.multiple_of(r * _RB, _RB), _RB)
            t = _dot(xb[rows, :], wb[:, cols])
            if part == 0:
                store_groups(q_s, cc, rows, _phi(t).astype(bf16))
            elif part == 1:
                store_groups(k_s, cc, rows, _phi(t).astype(bf16))
            else:
                store_groups(vb_s, cc, rows, t.astype(bf16))
            return carry

        lax.fori_loop(0, nr, proj_b, 0)

    rid = lax.broadcasted_iota(jnp.int32, (_LANES, 2 * _LANES), 0)
    cid = lax.broadcasted_iota(jnp.int32, (_LANES, 2 * _LANES), 1)
    same_head = rid // dh == (cid % _LANES) // dh

    def lin_group(g, carry):
        v1 = jnp.concatenate([vb_s[g], jnp.ones((S, _LANES), bf16)], axis=1)
        kvz = _dot(k_s[g], v1, _TN)
        kvz = jnp.where(same_head, kvz, 0.0).astype(bf16)
        nd = _dot(q_s[g], kvz)
        o = nd[:, :_LANES] / (nd[:, _LANES:] + 1e-6)
        xa[:, pl.ds(pl.multiple_of(g * _LANES, _LANES), _LANES)] = o.astype(bf16)
        return carry

    lax.fori_loop(0, ngrp, lin_group, 0)

    rest[3].wait()
    for r in range(nr):
        rows = slice(r * _RB, (r + 1) * _RB)
        out_s[rows, D:2 * D] = _dot(xa[rows, :], wob[...]).astype(bf16)
        out_copy(1, r).start()

    for half in range(2):
        for r in range(nr):
            out_copy(half, r).wait()


@jax.jit
def pallas_concat_heads__mha_block__linear_attn_block__prompt_kernel(
    A_x: jax.Array,
    A_wqkv: jax.Array,
    A_wo: jax.Array,
    B_x: jax.Array,
    B_wqkv: jax.Array,
    B_wo: jax.Array,
):
    B, S, D = A_x.shape
    assert B == 1 and B_x.shape == A_x.shape
    bf16, f32 = jnp.bfloat16, jnp.float32
    ngrp = D // _LANES
    n_in = S // _RB + 3 * D // _CB + 4
    any_spec = pl.BlockSpec(memory_space=pl.ANY)
    out = pl.pallas_call(
        _kernel,
        out_shape=jax.ShapeDtypeStruct((S, 2 * D), bf16),
        in_specs=[any_spec] * 6,
        out_specs=any_spec,
        scratch_shapes=[
            pltpu.VMEM((S, D), bf16),
            pltpu.VMEM((D, 3 * D), bf16),
            pltpu.VMEM((D, D), bf16),
            pltpu.VMEM((S, D), bf16),
            pltpu.VMEM((D, 3 * D), bf16),
            pltpu.VMEM((D, D), bf16),
            pltpu.VMEM((ngrp, S, _LANES), bf16),
            pltpu.VMEM((ngrp, S, _LANES), bf16),
            pltpu.VMEM((D, S), bf16),
            pltpu.VMEM((D, S), bf16),
            pltpu.VMEM((S, _BQ), f32),
            pltpu.VMEM((S, _BQ), f32),
            pltpu.VMEM((ngrp, S, _LANES), bf16),
            pltpu.VMEM((S, 2 * D), bf16),
            pltpu.SemaphoreType.DMA((n_in,)),
            pltpu.SemaphoreType.DMA((2 * (S // _RB),)),
        ],
        compiler_params=pltpu.CompilerParams(vmem_limit_bytes=110 * 1024 * 1024),
    )(A_x.reshape(S, D), A_wqkv, A_wo, B_x.reshape(S, D), B_wqkv, B_wo)
    return out.reshape(B, S, 2 * D)
```

```python
import math

import jax
import jax.numpy as jnp
from jax import lax
import jax.experimental.pallas as pl
import jax.experimental.pallas.tpu as pltpu

_H = 32
_LANES = 128
_BQ = 512
_CK = 128
_RB = 512
_CB = 512
_TB = 256
_DELTA = 2
_LA = 2
_SUM = "tree"
_ORDER = "pq"
_STAGED = 1
_SCOPES = 0

_NN = (((1,), (0,)), ((), ()))
_NT = (((1,), (1,)), ((), ()))
_TN = (((0,), (0,)), ((), ()))
_TT = (((0,), (1,)), ((), ()))


def _dot(a, b, dims=_NN):
    return lax.dot_general(a, b, dims, preferred_element_type=jnp.float32)


def _phi(t):
    return jnp.where(t > 0, t + 1.0, jnp.exp(t)) + 1e-6


def _tree_sum(p, lo, hi):
    if hi - lo == 1:
        return p[lo]
    mid = (lo + hi) // 2
    return _tree_sum(p, lo, mid) + _tree_sum(p, mid, hi)


class _Null:
    def __enter__(self): return self
    def __exit__(self, *a): return False


def _scope(name):
    return jax.named_scope(name) if _SCOPES else _Null()


def _kernel(xa_hbm, wa_hbm, woa_hbm, xb_hbm, wb_hbm, wob_hbm, out_hbm,
            xa, wa, woa, xb, wb, wob,
            qt_s, k_s, vt_s, ot_s, s_s, qb_s, vb_s, out_s,
            in_sems, out_sems):
    S, D = xa.shape
    dh = D // _H
    hpg = _LANES // dh
    ngrp = D // _LANES
    nr = S // _RB
    ncb = D // _CB
    gpb = _CB // _LANES
    nq = S // _BQ
    nc = S // _CK
    bf16, f32 = jnp.bfloat16, jnp.float32

    def x_copy(r):
        rows = pl.ds(r * _RB, _RB)
        return pltpu.make_async_copy(xa_hbm.at[rows, :], xa.at[rows, :], in_sems.at[r])

    def w_copy(c):
        cols = pl.ds(c * _CB, _CB)
        return pltpu.make_async_copy(wa_hbm.at[:, cols], wa.at[:, cols], in_sems.at[nr + c])

    rest = [
        pltpu.make_async_copy(src, dst, in_sems.at[nr + 3 * ncb + i])
        for i, (src, dst) in enumerate(
            [(woa_hbm, woa), (xb_hbm, xb), (wb_hbm, wb), (wob_hbm, wob)])
    ]
    x_copy(0).start()
    w_copy(ncb).start()
    if not _STAGED:
        for r in range(1, nr):
            x_copy(r).start()
        for c in list(range(ncb + 1, 3 * ncb)) + list(range(ncb)):
            w_copy(c).start()
        for cp in rest:
            cp.start()

    qscale = (dh ** -0.5) * math.log2(math.e)

    def store_groups(dst, c, rows, val):
        for g in range(gpb):
            dst[c * gpb + g, rows, :] = val[:, g * _LANES:(g + 1) * _LANES]

    with _scope("projA"):
        for cc in range(ncb):
            c = ncb + cc
            cols = slice(c * _CB, (c + 1) * _CB)
            w_copy(c).wait()

            def proj_k(r, carry, cc=cc, cols=cols):
                rows = pl.ds(pl.multiple_of(r * _RB, _RB), _RB)
                store_groups(k_s, cc, rows, _dot(xa[rows, :], wa[:, cols]).astype(bf16))
                return carry

            if cc == 0:
                for r in range(nr):
                    x_copy(r).wait()
                    if _STAGED and r == 0:
                        for r2 in range(1, nr):
                            x_copy(r2).start()
                        for c2 in list(range(ncb + 1, 3 * ncb)) + list(range(ncb)):
                            w_copy(c2).start()
                    if _STAGED and r == nr - 1:
                        for cp in rest:
                            cp.start()
                    proj_k(r, 0)
            else:
                lax.fori_loop(0, nr, proj_k, 0)

        for part, dst, scale in ((2, vt_s, None), (0, qt_s, qscale)):
            for cc in range(ncb):
                w_copy(part * ncb + cc).wait()

            def proj_t(j, carry, part=part, dst=dst, scale=scale):
                cols = pl.ds(pl.multiple_of(part * D + j * _TB, _TB), _TB)
                t = _dot(wa[:, cols], xa[...], _TT)
                if scale is not None:
                    t = t * scale
                dst[pl.ds(pl.multiple_of(j * _TB, _TB), _TB), :] = t.astype(bf16)
                return carry

            lax.fori_loop(0, D // _TB, proj_t, 0)

    n_it = ngrp * nq

    def qk(it, hh, c, slot):
        g = it // nq
        qi = it % nq
        q = qt_s[pl.ds(pl.multiple_of(g * _LANES + hh * dh, dh), dh),
                 pl.ds(pl.multiple_of(qi * _BQ, _BQ), _BQ)]
        parts = []
        if hh > 0:
            parts.append(jnp.zeros((dh * hh, _BQ), bf16))
        parts.append(q)
        if hh < hpg - 1:
            parts.append(jnp.zeros((dh * (hpg - 1 - hh), _BQ), bf16))
        ks = slice(c * _CK, (c + 1) * _CK)
        st = _dot(k_s[g, ks, :], jnp.concatenate(parts, axis=0))
        s_s[slot, ks, :] = st
        return jnp.max(st.reshape(_CK // 8, 8, _BQ), axis=0)

    def final_max(m8):
        return jnp.broadcast_to(jnp.max(m8, axis=0, keepdims=True), (8, _BQ))

    def attn_body(it, carry):
        m_cur, m8 = carry
        nxt = jnp.minimum(it + 1, n_it - 1)
        g = it // nq
        qi = it % nq
        zero = it >> 20
        slots = (zero, 1 - zero)

        def load(t):
            hh, c = divmod(t, nc)
            return s_s[slots[hh % 2], c * _CK:(c + 1) * _CK, :]

        ahead = [load(t) for t in range(_LA)]
        m_nxt = l8 = lm = acc = None
        for t in range(hpg * nc):
            hh, c = divmod(t, nc)
            uh, uc = divmod(t + nc + _DELTA, nc)
            if c == 0:
                l8 = lm = acc = None
            ks = slice(c * _CK, (c + 1) * _CK)
            hs = pl.ds(pl.multiple_of(g * _LANES + hh * dh, dh), dh)
            p = jnp.exp2(ahead.pop(0).reshape(_CK // 8, 8, _BQ) - m_cur[None])
            vt = vt_s[hs, ks]
            ll = _tree_sum(p, 0, _CK // 8)
            l8 = ll if l8 is None else l8 + ll
            a = _dot(vt, p.reshape(_CK, _BQ).astype(bf16))
            acc = a if acc is None else acc + a
            if t + _LA < hpg * nc:
                ahead.append(load(t + _LA))
            mm = qk(it if uh < hpg else nxt, uh % hpg, uc, slots[uh % 2])
            m8 = mm if uc == 0 else jnp.maximum(m8, mm)
            if uc == nc - 1:
                m_nxt = final_max(m8)
            if c == nc - 1:
                l = 0.0
                if l8 is not None:
                    l = l + jnp.sum(l8, axis=0, keepdims=True)
                if lm is not None:
                    l = l + lm[0:1]
                ot_s[hs, pl.ds(pl.multiple_of(qi * _BQ, _BQ), _BQ)] = (acc / l).astype(bf16)
                m_cur = m_nxt
        return m_cur, m8

    with _scope("attn"):
        m8 = None
        for c in range(nc):
            mm = qk(0, 0, c, 0)
            m8 = mm if c == 0 else jnp.maximum(m8, mm)
        m0 = final_max(m8)
        for c in range(_DELTA):
            mm = qk(0, 1, c, 1)
            m8 = mm if c == 0 else jnp.maximum(m8, mm)
        lax.fori_loop(0, n_it, attn_body, (m0, m8))

    def out_copy(half, r):
        rows = pl.ds(r * _RB, _RB)
        cols = pl.ds(half * D, D)
        return pltpu.make_async_copy(out_s.at[rows, cols], out_hbm.at[rows, cols],
                                     out_sems.at[half * nr + r])

    with _scope("outA"):
        rest[0].wait()
        for r in range(nr):
            rows = slice(r * _RB, (r + 1) * _RB)
            out_s[rows, 0:D] = _dot(ot_s[:, rows], woa[...], _TN).astype(bf16)
            out_copy(0, r).start()

    with _scope("projB"):
        rest[1].wait()
        rest[2].wait()
        zs = []
        for c in range(3 * ncb):
            part, cc = divmod(c, ncb)
            cols = slice(c * _CB, (c + 1) * _CB)

            def proj_b(r, z8, part=part, cc=cc, cols=cols):
                rows = pl.ds(pl.multiple_of(r * _RB, _RB), _RB)
                t = _dot(xb[rows, :], wb[:, cols])
                if part == 0:
                    store_groups(qb_s, cc, rows, _phi(t).astype(bf16))
                elif part == 1:
                    pk = _phi(t)
                    store_groups(k_s, cc, rows, pk.astype(bf16))
                    z8 = z8 + jnp.sum(pk.reshape(_RB // 8, 8, _CB), axis=0)
                else:
                    store_groups(vb_s, cc, rows, t.astype(bf16))
                return z8

            z8 = lax.fori_loop(0, nr, proj_b, jnp.zeros((8, _CB), f32))
            if part == 1:
                zs.append(jnp.sum(z8, axis=0, keepdims=True))

    with _scope("linB"):
        rid = lax.broadcasted_iota(jnp.int32, (_LANES, _LANES), 0)
        cid = lax.broadcasted_iota(jnp.int32, (_LANES, _LANES), 1)
        same_head = rid // dh == cid // dh
        for g in range(ngrp):
            cc, gg = divmod(g, gpb)
            z = zs[cc][:, gg * _LANES:(gg + 1) * _LANES]
            kvt = _dot(vb_s[g], k_s[g], _TN)
            rt = jnp.concatenate([jnp.where(same_head, kvt, 0.0),
                                  jnp.where(same_head, z, 0.0)], axis=0).astype(bf16)
            nd = _dot(qb_s[g], rt, _NT)
            o = nd[:, :_LANES] / (nd[:, _LANES:] + 1e-6)
            xa[:, g * _LANES:(g + 1) * _LANES] = o.astype(bf16)

    with _scope("outB"):
        rest[3].wait()
        for r in range(nr):
            rows = slice(r * _RB, (r + 1) * _RB)
            out_s[rows, D:2 * D] = _dot(xa[rows, :], wob[...]).astype(bf16)
            out_copy(1, r).start()

        for half in range(2):
            for r in range(nr):
                out_copy(half, r).wait()


@jax.jit
def pallas_concat_heads__mha_block__linear_attn_block__prompt_kernel(
    A_x: jax.Array,
    A_wqkv: jax.Array,
    A_wo: jax.Array,
    B_x: jax.Array,
    B_wqkv: jax.Array,
    B_wo: jax.Array,
):
    B, S, D = A_x.shape
    assert B == 1 and B_x.shape == A_x.shape
    bf16, f32 = jnp.bfloat16, jnp.float32
    ngrp = D // _LANES
    n_in = S // _RB + 3 * D // _CB + 4
    any_spec = pl.BlockSpec(memory_space=pl.ANY)
    out = pl.pallas_call(
        _kernel,
        out_shape=jax.ShapeDtypeStruct((S, 2 * D), bf16),
        in_specs=[any_spec] * 6,
        out_specs=any_spec,
        scratch_shapes=[
            pltpu.VMEM((S, D), bf16),
            pltpu.VMEM((D, 3 * D), bf16),
            pltpu.VMEM((D, D), bf16),
            pltpu.VMEM((S, D), bf16),
            pltpu.VMEM((D, 3 * D), bf16),
            pltpu.VMEM((D, D), bf16),
            pltpu.VMEM((D, S), bf16),
            pltpu.VMEM((ngrp, S, _LANES), bf16),
            pltpu.VMEM((D, S), bf16),
            pltpu.VMEM((D, S), bf16),
            pltpu.VMEM((2, S, _BQ), f32),
            pltpu.VMEM((ngrp, S, _LANES), bf16),
            pltpu.VMEM((ngrp, S, _LANES), bf16),
            pltpu.VMEM((S, 2 * D), bf16),
            pltpu.SemaphoreType.DMA((n_in,)),
            pltpu.SemaphoreType.DMA((2 * (S // _RB),)),
        ],
        compiler_params=pltpu.CompilerParams(vmem_limit_bytes=110 * 1024 * 1024),
    )(A_x.reshape(S, D), A_wqkv, A_wo, B_x.reshape(S, D), B_wqkv, B_wo)
    return out.reshape(B, S, 2 * D)
```

```python
import math

import jax
import jax.numpy as jnp
from jax import lax
import jax.experimental.pallas as pl
import jax.experimental.pallas.tpu as pltpu

_H = 32
_LANES = 128
_BQ = 512
_CK = 128
_RB = 512
_CB = 512
_TB = 256
_DELTA = 2
_LA = 2
_UNR = 2
_PEEL = 2
_OUT_ROWS = ((0, 1024), (1024, 1024), (0, 1024), (1024, 512), (1536, 256), (1792, 128), (1920, 128))
_SCOPES = 0

_NN = (((1,), (0,)), ((), ()))
_TN = (((0,), (0,)), ((), ()))
_TT = (((0,), (1,)), ((), ()))


def _dot(a, b, dims=_NN):
    return lax.dot_general(a, b, dims, preferred_element_type=jnp.float32)


def _phi(t):
    return jnp.where(t > 0, t + 1.0, jnp.exp(t)) + 1e-6


def _tree_sum(p, lo, hi):
    if hi - lo == 1:
        return p[lo]
    mid = (lo + hi) // 2
    return _tree_sum(p, lo, mid) + _tree_sum(p, mid, hi)


class _Null:
    def __enter__(self): return self
    def __exit__(self, *a): return False


def _scope(name):
    return jax.named_scope(name) if _SCOPES else _Null()


def _block(i, size):
    if isinstance(i, int):
        return slice(i * size, (i + 1) * size)
    return pl.ds(pl.multiple_of(i * size, size), size)


def _kernel(xa_hbm, wa_hbm, woa_hbm, xb_hbm, wb_hbm, wob_hbm, out_hbm,
            xa, wa, woa, xb, wb, wob,
            vq_s, k_s, ot_s, s_s, out_s,
            x_sems, w_sems, rest_sems, out_sems):
    S, D = xa.shape
    dh = D // _H
    hpg = _LANES // dh
    ngrp = D // _LANES
    nr = S // _RB
    ncb = D // _CB
    gpb = _CB // _LANES
    nq = S // _BQ
    nc = S // _CK
    nx = S // _TB
    nw = D // _TB
    bf16, f32 = jnp.bfloat16, jnp.float32

    def x_copy(i):
        rows = pl.ds(pl.multiple_of(i * _TB, _TB), _TB)
        return pltpu.make_async_copy(xa_hbm.at[rows, :], xa.at[rows, :], x_sems.at[i])

    def w_copy(i):
        cols = pl.ds(pl.multiple_of(i * _TB, _TB), _TB)
        return pltpu.make_async_copy(wa_hbm.at[:, cols], wa.at[:, cols], w_sems.at[i])

    later = [
        pltpu.make_async_copy(src, dst, rest_sems.at[i])
        for i, (src, dst) in enumerate(
            [(xb_hbm, xb), (wb_hbm, wb), (woa_hbm, woa), (wob_hbm, wob)])
    ]
    w0 = _CB // _TB
    x_copy(0).start()
    for i in range(w0):
        w_copy(nw + i).start()
    x_copy(1).start()

    def store_k(g0, rows, val):
        for g in range(val.shape[1] // _LANES):
            k_s[g0 + g, rows, :] = val[:, _block(g, _LANES)].astype(bf16)

    def proj_k_first(i, carry):
        @pl.when(i == 0)
        def _():
            x_copy(0).wait()

        w_copy(nw + i).wait()
        store_k(i * (_TB // _LANES), _block(0, _TB),
                _dot(xa[_block(0, _TB), :], wa[:, _block(nw + i, _TB)]))
        return carry

    def proj_k(i, carry):
        x_copy(i).wait()

        @pl.when(i + 1 < nx)
        def _():
            x_copy(i + 1).start()

        w_copy((2 * nw + i - 1) % (3 * nw)).start()
        store_k(0, _block(i, _TB), _dot(xa[_block(i, _TB), :], wa[:, _block(ncb, _CB)]))
        return carry

    w_left = list(range(nx - 1 - nw, nw)) + list(range(nw + w0, 2 * nw))

    def proj_v(j, carry):
        w_copy(2 * nw + j).wait()

        @pl.when(j == 0)
        def _():
            for n in w_left:
                w_copy(n).start()

        @pl.when(j == 1)
        def _():
            for cp in later:
                cp.start()

        vq_s[_block(j, _TB), :] = _dot(wa[:, _block(2 * nw + j, _TB)], xa[...], _TT).astype(bf16)
        return carry

    with _scope("projA"):
        lax.fori_loop(0, w0, proj_k_first, 0)
        lax.fori_loop(1, nx, proj_k, 0)
        lax.fori_loop(0, nw, proj_v, 0)
        for n in list(range(nw)) + list(range(nw + w0, 2 * nw)):
            w_copy(n).wait()
        for cc in range(1, ncb):
            for r in range(nr):
                store_k(cc * gpb, _block(r, _RB),
                        _dot(xa[_block(r, _RB), :], wa[:, _block(ncb + cc, _CB)]))
        qscale = (dh ** -0.5) * math.log2(math.e)
        for j in range(nw):
            q = _dot(wa[:, _block(j, _TB)], xa[...], _TT) * qscale
            vq_s[_block(nw + j, _TB), :] = q.astype(bf16)

    n_steps = ngrp * nq

    def scores(step, hh, c, slot):
        qi, g = step // ngrp, step % ngrp
        q = vq_s[_block(_H + g * hpg + hh, dh), _block(qi, _BQ)]
        parts = [jnp.zeros((dh * hh, _BQ), bf16), q, jnp.zeros((dh * (hpg - 1 - hh), _BQ), bf16)]
        q = jnp.concatenate([x for x in parts if x.shape[0]], axis=0)
        st = _dot(k_s[g, _block(c, _CK), :], q)
        s_s[slot, _block(c, _CK), :] = st
        return jnp.max(st.reshape(_CK // 8, 8, _BQ), axis=0)

    def final_max(m8):
        return jnp.broadcast_to(jnp.max(m8, axis=0, keepdims=True), (8, _BQ))

    def attention(first, count, carry, last):
        m_cur, m8, slot0 = carry
        slots = (slot0, 1 - slot0)
        nt = count * hpg * nc

        def load(t):
            hh, c = divmod(t, nc)
            return s_s[slots[hh % 2], _block(c, _CK), :]

        ahead = [load(t) for t in range(_LA)]
        for t in range(nt):
            hh, c = divmod(t, nc)
            step = first + hh // hpg
            head = (step % ngrp) * hpg + hh % hpg
            p = jnp.exp2(ahead.pop(0).reshape(_CK // 8, 8, _BQ) - m_cur[None])
            ll = _tree_sum(p, 0, _CK // 8)
            l8 = ll if c == 0 else l8 + ll
            pv = _dot(vq_s[_block(head, dh), _block(c, _CK)], p.reshape(_CK, _BQ).astype(bf16))
            acc = pv if c == 0 else acc + pv
            if t + _LA < nt:
                ahead.append(load(t + _LA))
            uh, uc = divmod(t + nc + _DELTA, nc)
            if not (last and uh >= count * hpg):
                mm = scores(first + uh // hpg, uh % hpg, uc, slots[uh % 2])
                m8 = mm if uc == 0 else jnp.maximum(m8, mm)
                if uc == nc - 1:
                    m_nxt = final_max(m8)
            if c == nc - 1:
                o = acc / jnp.sum(l8, axis=0, keepdims=True)
                ot_s[_block(head, dh), _block(step // ngrp, _BQ)] = o.astype(bf16)
                m_cur = m_nxt
        return m_cur, m8

    def attention_loop(j, carry):
        m_cur, m8 = attention(j * _UNR, _UNR, (carry[0], carry[1], j >> 20), False)
        return m_cur, m8, j >> 20

    with _scope("attn"):
        for c in range(nc):
            mm = scores(0, 0, c, 0)
            m8 = mm if c == 0 else jnp.maximum(m8, mm)
        m0 = final_max(m8)
        for c in range(_DELTA):
            mm = scores(0, 1, c, 1)
            m8 = mm if c == 0 else jnp.maximum(m8, mm)
        carry = lax.fori_loop(0, (n_steps - _PEEL) // _UNR, attention_loop, (m0, m8, jnp.int32(0)))
    with _scope("peel"):
        attention(n_steps - _PEEL, _PEEL, carry, True)

    with _scope("B"):
        for cp in later:
            cp.wait()
        z = []
        for cc in range(ncb):
            for r in range(nr):
                pk = _phi(_dot(xb[_block(r, _RB), :], wb[:, _block(ncb + cc, _CB)]))
                xa[_block(r, _RB), _block(cc, _CB)] = pk.astype(bf16)
                zr = jnp.sum(pk.reshape(_RB // 8, 8, _CB), axis=0)
                z8 = zr if r == 0 else z8 + zr
            z.append(jnp.sum(z8, axis=0, keepdims=True))
        for j in range(nw):
            pq = _phi(_dot(wb[:, _block(j, _TB)], xb[...], _TT))
            vq_s[_block(nw + j, _TB), :] = pq.astype(bf16)

        own_head = (lax.broadcasted_iota(jnp.int32, (8, _LANES), 0)
                    == lax.broadcasted_iota(jnp.int32, (8, _LANES), 1) // dh)
        same_head = (lax.broadcasted_iota(jnp.int32, (_LANES, _LANES), 0) // dh
                     == lax.broadcasted_iota(jnp.int32, (_LANES, _LANES), 1) // dh)

        def normalise(g, cols):
            cc, gg = divmod(g, gpb)
            zsel = jnp.where(own_head, z[cc][:, _block(gg, _LANES)], 0.0)
            pq = vq_s[_block(ngrp + g, _LANES), cols]
            inv = 1.0 / (_dot(zsel, pq) + 1e-6)
            for hh in range(hpg):
                pn = pq[_block(hh, dh)].astype(f32) * inv[hh:hh + 1]
                vq_s[_block(g * hpg + hh, dh), cols] = pn.astype(bf16)

        def fold(g, kx):
            kv = jnp.where(same_head, _dot(kx, wb[:, _block(2 * ngrp + g, _LANES)]), 0.0)
            m = _dot(kv.astype(bf16), wob[_block(g, _LANES), :])
            wa[_block(g, _LANES), 0:D] = m.astype(bf16)

        to_fold = []
        to_norm = [(g, _block(i, _CB)) for g in range(ngrp) for i in range(S // _CB)]
        for cc in range(ncb):
            for c in range(nc):
                part = _dot(xa[_block(c, _CK), _block(cc, _CB)], xb[_block(c, _CK), :], _TN)
                kx = part if c == 0 else kx + part
                normalise(*to_norm.pop(0))
                if to_fold and c % 2 == 1:
                    fold(*to_fold.pop(0))
            kx = kx.astype(bf16)
            to_fold += [(cc * gpb + gg, kx[_block(gg, _LANES)]) for gg in range(gpb)]
        assert not to_norm

    with _scope("out"):
        out_copies = []
        done = 0
        for start, size in _OUT_ROWS:
            half = done // S
            rows = slice(start, start + size)
            src, w = (ot_s, woa) if half == 0 else (vq_s, wa)
            out_s[rows, _block(half, D)] = _dot(src[0:D, rows], w[:, 0:D], _TN).astype(bf16)
            while to_fold:
                fold(*to_fold.pop(0))
            idx = (pl.ds(start, size), pl.ds(half * D, D))
            out_copies.append(pltpu.make_async_copy(
                out_s.at[idx], out_hbm.at[idx], out_sems.at[len(out_copies)]))
            out_copies[-1].start()
            done += size
        assert done == 2 * S
        for cp in out_copies:
            cp.wait()


@jax.jit
def pallas_concat_heads__mha_block__linear_attn_block__prompt_kernel(
    A_x: jax.Array,
    A_wqkv: jax.Array,
    A_wo: jax.Array,
    B_x: jax.Array,
    B_wqkv: jax.Array,
    B_wo: jax.Array,
):
    B, S, D = A_x.shape
    assert B == 1 and B_x.shape == A_x.shape
    bf16, f32 = jnp.bfloat16, jnp.float32
    any_spec = pl.BlockSpec(memory_space=pl.ANY)
    out = pl.pallas_call(
        _kernel,
        out_shape=jax.ShapeDtypeStruct((S, 2 * D), bf16),
        in_specs=[any_spec] * 6,
        out_specs=any_spec,
        scratch_shapes=[
            pltpu.VMEM((S, D), bf16),
            pltpu.VMEM((D, 3 * D), bf16),
            pltpu.VMEM((D, D), bf16),
            pltpu.VMEM((S, D), bf16),
            pltpu.VMEM((D, 3 * D), bf16),
            pltpu.VMEM((D, D), bf16),
            pltpu.VMEM((2 * D, S), bf16),
            pltpu.VMEM((D // _LANES, S, _LANES), bf16),
            pltpu.VMEM((D, S), bf16),
            pltpu.VMEM((2, S, _BQ), f32),
            pltpu.VMEM((S, 2 * D), bf16),
            pltpu.SemaphoreType.DMA((S // _TB,)),
            pltpu.SemaphoreType.DMA((3 * D // _TB,)),
            pltpu.SemaphoreType.DMA((4,)),
            pltpu.SemaphoreType.DMA((len(_OUT_ROWS),)),
        ],
        compiler_params=pltpu.CompilerParams(vmem_limit_bytes=110 * 1024 * 1024),
    )(A_x.reshape(S, D), A_wqkv, A_wo, B_x.reshape(S, D), B_wqkv, B_wo)
    return out.reshape(B, S, 2 * D)
```

```python
import math

import jax
import jax.numpy as jnp
from jax import lax
import jax.experimental.pallas as pl
import jax.experimental.pallas.tpu as pltpu

_H = 32
_LANES = 128
_SUBLANES = 8
_BQ = 512
_CK = 128
_RB = 512
_CB = 512
_TB = 256
_DELTA = 2
_AHEAD = 2
_UNROLL = 2
_OUT_ROWS = (1280, 512, 256)

_NN = (((1,), (0,)), ((), ()))
_TN = (((0,), (0,)), ((), ()))
_TT = (((0,), (1,)), ((), ()))


def _dot(a, b, dims=_NN):
    return lax.dot_general(a, b, dims, preferred_element_type=jnp.float32)


def _phi(t):
    return jnp.where(t > 0, t + 1.0, jnp.exp(t)) + 1e-6


def _tree_sum(p, lo, hi):
    if hi - lo == 1:
        return p[lo]
    mid = (lo + hi) // 2
    return _tree_sum(p, lo, mid) + _tree_sum(p, mid, hi)


def _block(i, size):
    if isinstance(i, int):
        return slice(i * size, (i + 1) * size)
    return pl.ds(pl.multiple_of(i * size, size), size)


def _kernel(xa_hbm, wa_hbm, woa_hbm, xb_hbm, wb_hbm, wob_hbm, out_hbm,
            xa, wa, wo_s, xb, wb, wob,
            t_s, k_s, kt_s, o_s, s_s, z_s, out_s,
            x_sems, w_sems, rest_sems, out_sems):
    S, D = xa.shape
    dh = D // _H
    hpg = _LANES // dh
    ngrp = D // _LANES
    nr = S // _RB
    ncb = D // _CB
    gpb = _CB // _LANES
    nq = S // _BQ
    nc = S // _CK
    nx = S // _TB
    nw = D // _TB
    w0 = _CB // _TB
    bf16, f32 = jnp.bfloat16, jnp.float32

    def x_copy(i):
        rows = pl.ds(pl.multiple_of(i * _TB, _TB), _TB)
        return pltpu.make_async_copy(xa_hbm.at[rows, :], xa.at[rows, :], x_sems.at[i])

    def w_copy(i):
        cols = pl.ds(pl.multiple_of(i * _TB, _TB), _TB)
        return pltpu.make_async_copy(wa_hbm.at[:, cols], wa.at[:, cols], w_sems.at[i])

    later = [
        pltpu.make_async_copy(src, dst, rest_sems.at[i])
        for i, (src, dst) in enumerate(
            [(xb_hbm, xb), (wb_hbm, wb), (woa_hbm, wo_s.at[0]), (wob_hbm, wob)])
    ]
    x_copy(0).start()
    for i in range(w0):
        w_copy(nw + i).start()
    x_copy(1).start()

    def store_k(g0, rows, val):
        for g in range(val.shape[1] // _LANES):
            k_s[g0 + g, rows, :] = val[:, _block(g, _LANES)].astype(bf16)

    def proj_k_first(i, carry):
        @pl.when(i == 0)
        def _():
            x_copy(0).wait()

        w_copy(nw + i).wait()
        store_k(i * (_TB // _LANES), _block(0, _TB),
                _dot(xa[_block(0, _TB), :], wa[:, _block(nw + i, _TB)]))
        return carry

    def proj_k(i, carry):
        x_copy(i).wait()

        @pl.when(i + 1 < nx)
        def _():
            x_copy(i + 1).start()

        w_copy((nw + w0 + i - 1) % (3 * nw)).start()
        store_k(0, _block(i, _TB), _dot(xa[_block(i, _TB), :], wa[:, _block(ncb, _CB)]))
        return carry

    qscale = (dh ** -0.5) * math.log2(math.e)

    def proj_vq(i, carry):
        first = (1 - i) * 2 * nw
        for j in range(nw):
            w_copy(first + j).wait()
        scale = jnp.where(i == 0, 1.0, qscale).astype(f32)
        for j in range(nw):
            t = _dot(wa[:, _block(first + j, _TB)], xa[...], _TT) * scale
            t_s[_block(i * nw + j, _TB), :] = t.astype(bf16)
        for cc in range(1, ncb):
            for r in range(nr // 2):
                rows = _block(i * (nr // 2) + r, _RB)
                store_k(cc * gpb, rows, _dot(xa[rows, :], wa[:, _block(ncb + cc, _CB)]))
        return carry

    lax.fori_loop(0, w0, proj_k_first, 0)
    lax.fori_loop(1, nx, proj_k, 0)
    for n in range(nw + w0 + nx - 1, 4 * nw):
        w_copy(n % (3 * nw)).start()
    for cp in later:
        cp.start()
    for n in range(nw + w0, 2 * nw):
        w_copy(n).wait()
    lax.fori_loop(0, 2, proj_vq, 0)

    n_steps = ngrp * nq

    def scores(step, hh, c, slot):
        qi, g = step // ngrp, step % ngrp
        q = t_s[_block(_H + g * hpg + hh, dh), _block(qi, _BQ)]
        parts = [jnp.zeros((dh * hh, _BQ), bf16), q, jnp.zeros((dh * (hpg - 1 - hh), _BQ), bf16)]
        q = jnp.concatenate([x for x in parts if x.shape[0]], axis=0)
        st = _dot(k_s[g, _block(c, _CK), :], q)
        s_s[slot, _block(c, _CK), :] = st
        return jnp.max(st.reshape(_CK // _SUBLANES, _SUBLANES, _BQ), axis=0)

    def final_max(m8):
        return jnp.broadcast_to(jnp.max(m8, axis=0, keepdims=True), (_SUBLANES, _BQ))

    def attention(first, count, carry, filler=None):
        m_cur, m8, slot0 = carry
        slots = (slot0, 1 - slot0)
        nt = count * hpg * nc

        def load(t):
            hh, c = divmod(t, nc)
            return s_s[slots[hh % 2], _block(c, _CK), :]

        ahead = [load(t) for t in range(_AHEAD)]
        for t in range(nt):
            hh, c = divmod(t, nc)
            step = first + hh // hpg
            head = (step % ngrp) * hpg + hh % hpg
            p = jnp.exp2(ahead.pop(0).reshape(_CK // _SUBLANES, _SUBLANES, _BQ) - m_cur[None])
            for i in range(0, _CK // _SUBLANES, 8):
                ll = _tree_sum(p, i, i + 8)
                l8 = ll if c == 0 and i == 0 else l8 + ll
            pv = _dot(t_s[_block(head, dh), _block(c, _CK)], p.reshape(_CK, _BQ).astype(bf16))
            acc = pv if c == 0 else acc + pv
            if t + _AHEAD < nt:
                ahead.append(load(t + _AHEAD))
            uh, uc = divmod(t + nc + _DELTA, nc)
            if filler is not None and uh >= count * hpg:
                filler()
            else:
                mm = scores(first + uh // hpg, uh % hpg, uc, slots[uh % 2])
                m8 = mm if uc == 0 else jnp.maximum(m8, mm)
                if uc == nc - 1:
                    m_nxt = final_max(m8)
            if c == nc - 1:
                o = acc / jnp.sum(l8, axis=0, keepdims=True)
                o_s[0, _block(head, dh), _block(step // ngrp, _BQ)] = o.astype(bf16)
                m_cur = m_nxt
        return m_cur, m8

    def attention_loop(j, carry):
        m_cur, m8 = attention(j * _UNROLL, _UNROLL, (carry[0], carry[1], j >> 20))
        return m_cur, m8, j >> 20

    for c in range(nc):
        mm = scores(0, 0, c, 0)
        m8 = mm if c == 0 else jnp.maximum(m8, mm)
    m0 = final_max(m8)
    for c in range(_DELTA):
        mm = scores(0, 1, c, 1)
        m8 = mm if c == 0 else jnp.maximum(m8, mm)
    carry = lax.fori_loop(0, n_steps // _UNROLL - 1, attention_loop, (m0, m8, jnp.int32(0)))

    for cp in later:
        cp.wait()
    k_todo = [(j, r) for j in range(nw) for r in range(nr)]
    zp = [None] * nw

    def proj_kb():
        if k_todo:
            j, r = k_todo.pop(0)
            pk = _phi(_dot(wb[:, _block(nw + j, _TB)], xb[_block(r, _RB), :], _TT))
            kt_s[_block(j, _TB), _block(r, _RB)] = pk.astype(bf16)
            for i in range(_RB // _LANES):
                part = pk[:, _block(i, _LANES)]
                zp[j] = part if zp[j] is None else zp[j] + part
            if r == nr - 1:
                z = jnp.sum(zp[j], axis=1, keepdims=True)
                z_s[_block(j, _TB), :] = jnp.broadcast_to(z, (_TB, _LANES))

    attention(n_steps - _UNROLL, _UNROLL, carry, proj_kb)
    while k_todo:
        proj_kb()

    def proj_qb(i, carry):
        for jj in range(nw // 2):
            j = i * (nw // 2) + jj
            pq = _phi(_dot(wb[:, _block(j, _TB)], xb[...], _TT))
            zq = pq * jnp.concatenate([z_s[_block(j, _TB), :]] * (S // _LANES), axis=1)
            for h in range(_TB // dh):
                den = jnp.sum(zq[_block(h, dh)], axis=0, keepdims=True) + 1e-6
                pn = pq[_block(h, dh)] * (1.0 / den)
                o_s[1, _block(j * (_TB // dh) + h, dh), :] = pn.astype(bf16)
            wa[_block(j, _TB), 0:D] = _dot(kt_s[_block(j, _TB), :], xb[...]).astype(bf16)
        return carry

    lax.fori_loop(0, 2, proj_qb, 0)

    same_head = (lax.broadcasted_iota(jnp.int32, (_LANES, _LANES), 0) // dh
                 == lax.broadcasted_iota(jnp.int32, (_LANES, _LANES), 1) // dh)
    kvs = [_dot(wa[_block(g, _LANES), 0:D], wb[:, _block(2 * ngrp + g, _LANES)])
           for g in range(ngrp)]
    for g in range(ngrp):
        m = _dot(jnp.where(same_head, kvs[g], 0.0).astype(bf16), wob[_block(g, _LANES), :])
        wo_s[1, _block(g, _LANES), :] = m.astype(bf16)

    starts = [sum(_OUT_ROWS[:i]) for i in range(len(_OUT_ROWS))]

    def out_copy(half, i):
        idx = (pl.ds(starts[i], _OUT_ROWS[i]), pl.ds(pl.multiple_of(half * D, D), D))
        return pltpu.make_async_copy(out_s.at[idx], out_hbm.at[idx], out_sems.at[half, i])

    def out_proj(half, carry):
        for i, size in enumerate(_OUT_ROWS):
            rows = slice(starts[i], starts[i] + size)
            y = _dot(o_s[half, :, rows], wo_s[half], _TN)
            out_s[rows, _block(half, D)] = y.astype(bf16)
            out_copy(half, i).start()
        return carry

    lax.fori_loop(0, 2, out_proj, 0)
    for half in range(2):
        for i in range(len(_OUT_ROWS)):
            out_copy(half, i).wait()


@jax.jit
def pallas_concat_heads__mha_block__linear_attn_block__prompt_kernel(
    A_x: jax.Array,
    A_wqkv: jax.Array,
    A_wo: jax.Array,
    B_x: jax.Array,
    B_wqkv: jax.Array,
    B_wo: jax.Array,
):
    B, S, D = A_x.shape
    assert B == 1 and B_x.shape == A_x.shape
    assert (S, D) == (sum(_OUT_ROWS), 2 * _CB)
    bf16, f32 = jnp.bfloat16, jnp.float32
    any_spec = pl.BlockSpec(memory_space=pl.ANY)
    out = pl.pallas_call(
        _kernel,
        out_shape=jax.ShapeDtypeStruct((S, 2 * D), bf16),
        in_specs=[any_spec] * 6,
        out_specs=any_spec,
        scratch_shapes=[
            pltpu.VMEM((S, D), bf16),
            pltpu.VMEM((D, 3 * D), bf16),
            pltpu.VMEM((2, D, D), bf16),
            pltpu.VMEM((S, D), bf16),
            pltpu.VMEM((D, 3 * D), bf16),
            pltpu.VMEM((D, D), bf16),
            pltpu.VMEM((2 * D, S), bf16),
            pltpu.VMEM((D // _LANES, S, _LANES), bf16),
            pltpu.VMEM((D, S), bf16),
            pltpu.VMEM((2, D, S), bf16),
            pltpu.VMEM((2, S, _BQ), f32),
            pltpu.VMEM((D, _LANES), f32),
            pltpu.VMEM((S, 2 * D), bf16),
            pltpu.SemaphoreType.DMA((S // _TB,)),
            pltpu.SemaphoreType.DMA((3 * D // _TB,)),
            pltpu.SemaphoreType.DMA((4,)),
            pltpu.SemaphoreType.DMA((2, len(_OUT_ROWS))),
        ],
        compiler_params=pltpu.CompilerParams(vmem_limit_bytes=110 * 1024 * 1024),
    )(A_x.reshape(S, D), A_wqkv, A_wo, B_x.reshape(S, D), B_wqkv, B_wo)
    return out.reshape(B, S, 2 * D)
```
